```python
import os as _os
_os.environ.setdefault("JAX_PLATFORMS", "cpu")
import jax
import jax.numpy as jnp

def _softmax(x, axis=-1):
    return jax.nn.softmax(x, axis=axis)
def _gelu(x):
    return jax.nn.gelu(x, approximate=True)
def _silu(x):
    return jax.nn.silu(x)
def _sigmoid(x):
    return jax.nn.sigmoid(x)
def _layernorm(x, axis=-1, eps=1e-5):
    m = jnp.mean(x, axis=axis, keepdims=True)
    v = jnp.var(x, axis=axis, keepdims=True)
    return (x - m) / jnp.sqrt(v + eps)
def _scatter_add(tgt, idx, src, axis=0):
    return tgt.at[idx].add(src)
def _segment_sum(src, seg, n):
    return jax.ops.segment_sum(src, seg, n)
class _Rng:
    def __init__(self, key):
        self._k = key
    def _next(self):
        self._k, sub = jax.random.split(self._k)
        return sub
    def normal(self, shape):
        return jax.random.normal(self._next(), shape, dtype=jnp.bfloat16)
    def randint(self, lo, hi, shape):
        return jax.random.randint(self._next(), shape, lo, hi, dtype=jnp.int32)
    def uniform(self, shape, lo=0.0, hi=1.0):
        return jax.random.uniform(self._next(), shape, jnp.bfloat16, lo, hi)
    def permutation(self, n):
        return jax.random.permutation(self._next(), n)


kernel_name = 'standalone__gqa_block_cached__near_ridge'

def setup_inputs():
    _rng = _Rng(jax.random.key(int.from_bytes(__import__("os").urandom(4), "little")))
    _w = (lambda a: (lambda t: t.astype(jnp.bfloat16) if jnp.issubdtype(t.dtype, jnp.floating) else t)(jnp.asarray(a)))
    B, Sq, D = 8, 96, 448
    Hq, Hkv, Sk, Dh = 16, 8, 2048, 256
    assert Hq % Hkv == 0, (Hq, Hkv)
    return {
        "x": _w((lambda *s: _rng.normal(s) * 0.8)(B, Sq, D)),
        "k_cache": _w((lambda *s: _rng.normal(s) * 0.8)(B, Hkv, Sk, Dh)),
        "v_cache": _w((lambda *s: _rng.normal(s) * 0.05)(B, Hkv, Sk, Dh)),
        "wq": _w((lambda *s: _rng.normal(s) * 0.8)(D, Hq * Dh) * (D ** -0.5)),
        "wo": _w((lambda *s: _rng.normal(s) * 0.05)(Hq * Dh, D) * ((Hq * Dh) ** -0.5)),
    }

def reference(x, k_cache, v_cache, wq, wo):
    B, Sq, D = x.shape
    Hq, Dh = 16, 256
    Hkv = k_cache.shape[1]
    rep = Hq // Hkv
    q = (lambda x, *d: x.transpose(*d))((x @ wq).reshape(B, Sq, Hq, Dh), 0, 2, 1, 3)
    k = jnp.repeat(k_cache, rep, axis=1)
    v = jnp.repeat(v_cache, rep, axis=1)
    scores = jnp.einsum("bhqd,bhkd->bhqk", q, k) * (Dh ** -0.5)
    p = _softmax(scores, axis=-1)
    o = jnp.einsum("bhqk,bhkd->bhqd", p, v)
    return (lambda x, *d: x.transpose(*d))(o, 0, 2, 1, 3).reshape(B, Sq, Hq * Dh) @ wo
```

```python
import functools
import math
import jax
import jax.numpy as jnp
import jax.experimental.pallas as pl
import jax.experimental.pallas.tpu as pltpu

HQ, DH = 16, 256
NS = 8
CH = 512
DR = 88
LA = 4
LAK = 3
LAV = 3
ORDER = 'qp i fin i v0 i k0 i v1 i k1 i k2 i v2 i k3 i v3 i'
LOOP_ONLY = False
SCOPES = False
MIDWAIT = True
NT_DIMS = (((1,), (1,)), ((), ()))
QSCALE = (DH ** -0.5) * math.log2(math.e)

import contextlib
def scope(name):
    return jax.named_scope(name) if SCOPES else contextlib.nullcontext()


def _kernel(x_hbm, k_hbm, v_hbm, wq_hbm, wot_hbm, out_hbm,
            x_v, wq_v, wo_v, kbuf, vbuf, pa_ref, pb_ref, beta_ref, o_ref, acc_ref, ostage,
            xsem, wqsem, wosem, ksem, vsem, osem, *, B, Sq, D, Hkv, Sk, rep):
    T = B * Hkv
    W = rep * DH
    R = rep * Sq
    nch = Sk // CH
    DCH = 512
    ndc = Sk // DCH
    f32, bf16 = jnp.float32, jnp.bfloat16
    p_refs = (pa_ref, pb_ref)
    pieces = [(o, min(DR, DCH - o)) for o in range(0, DCH, DR)]

    def mod(x, n):
        assert n & (n - 1) == 0
        return x % n if isinstance(x, int) else jnp.bitwise_and(x, n - 1)

    def div(x, n):
        assert n & (n - 1) == 0
        return x // n if isinstance(x, int) else jax.lax.shift_right_logical(x, n.bit_length() - 1)

    def blk(t):
        return mod(t, B) * Hkv + div(t, B)

    def x_copy(part):
        if part == 0:
            return pltpu.make_async_copy(x_hbm.at[pl.ds(0, Sq)], x_v.at[pl.ds(0, Sq)], xsem.at[0])
        return pltpu.make_async_copy(x_hbm.at[pl.ds(Sq, (B - 1) * Sq)], x_v.at[pl.ds(Sq, (B - 1) * Sq)], xsem.at[1])

    WP = D // 4
    WR = WP // 2

    def w_part_start(hbm, buf, sem, h, part, prio):
        for j in range(2):
            r0 = part * WP + j * WR
            if not isinstance(r0, int):
                r0 = pl.multiple_of(r0, 8)
            pltpu.make_async_copy(hbm.at[pl.ds(r0, WR), pl.ds(h * W, W)], buf.at[h, pl.ds(r0, WR)], sem.at[h]).start(priority=prio)

    def wq_part(h, part, prio=0):
        w_part_start(wq_hbm, wq_v, wqsem, h, part, prio)

    def wo_part(h, part, prio=1):
        w_part_start(wot_hbm, wo_v, wosem, h, part, prio)

    def wq_wait(h):
        pltpu.make_async_copy(wq_v.at[h], wq_v.at[h], wqsem.at[h]).wait()

    def wo_wait(h):
        pltpu.make_async_copy(wo_v.at[h], wo_v.at[h], wosem.at[h]).wait()

    def k_chunk_start(t, c):
        slot = mod(t, NS)
        for o, n in pieces:
            r = c * DCH + o
            if not isinstance(r, int):
                r = pl.multiple_of(r, 8)
            pltpu.make_async_copy(k_hbm.at[blk(t), pl.ds(r, n)], kbuf.at[slot, pl.ds(r, n)], ksem.at[slot]).start(priority=0)

    def v_chunk_start(t, c, prio=1):
        slot = mod(t, NS)
        for o, n in pieces:
            r = c * DCH + o
            if not isinstance(r, int):
                r = pl.multiple_of(r, 8)
            pltpu.make_async_copy(v_hbm.at[blk(t), pl.ds(r, n)], vbuf.at[slot, pl.ds(r, n)], vsem.at[slot * ndc + c]).start(priority=prio)

    all_pieces = [(c, o, n) for c in range(ndc) for (o, n) in pieces]
    NI = ORDER.split().count('i')

    def k_piece(t, c, o, n):
        slot = mod(t, NS)
        r = c * DCH + o
        pltpu.make_async_copy(k_hbm.at[blk(t), pl.ds(r, n)], kbuf.at[slot, pl.ds(r, n)], ksem.at[slot]).start(priority=0)

    def v_piece(t, c, o, n):
        slot = mod(t, NS)
        r = c * DCH + o
        pltpu.make_async_copy(v_hbm.at[blk(t), pl.ds(r, n)], vbuf.at[slot, pl.ds(r, n)], vsem.at[slot * ndc + c]).start(priority=1)

    def k_wait(t):
        slot = mod(t, NS)
        pltpu.make_async_copy(kbuf.at[slot], kbuf.at[slot], ksem.at[slot]).wait()

    def v_wait_chunk(t, c):
        slot = mod(t, NS)
        dst = vbuf.at[slot, pl.ds(c * DCH, DCH)]
        pltpu.make_async_copy(dst, dst, vsem.at[slot * ndc + c]).wait()

    def v_wait(t):
        for c in range(ndc):
            v_wait_chunk(t, c)

    def out_copy(b):
        return pltpu.make_async_copy(ostage.at[b], out_hbm.at[b], osem.at[b])

    def rows_of(b):
        return pl.ds(b * Sq if isinstance(b, int) else pl.multiple_of(b * Sq, Sq), Sq)

    def qproj(t):
        b = mod(t, B)
        h = div(t, B)
        xb = x_v[rows_of(b), :]
        q = jnp.dot(xb, wq_v[h], preferred_element_type=f32)
        q = (q * QSCALE).astype(bf16)
        return jnp.concatenate([q[:, r * DH:(r + 1) * DH] for r in range(rep)], axis=0)

    def lane_fold(a, op):
        out = a[:, 0:128]
        for j in range(1, a.shape[1] // 128):
            out = op(out, a[:, j * 128:(j + 1) * 128])
        return out

    def qk_chunk(q2, t, par, c):
        k = kbuf[mod(t, NS), pl.ds(c * CH, CH), :]
        s = jax.lax.dot_general(q2, k, NT_DIMS, preferred_element_type=f32)
        mc = jnp.max(lane_fold(s, jnp.maximum), axis=-1, keepdims=True)
        p = jnp.exp2(s - mc)
        p_refs[par][:, c * CH:(c + 1) * CH] = p.astype(bf16)
        return jnp.broadcast_to(mc, (R, 128)), lane_fold(p, jnp.add)

    def betas(ms, ls):
        m = ms[0]
        for x in ms[1:]:
            m = jnp.maximum(m, x)
        al = [jnp.exp2(x - m) for x in ms]
        l = al[0] * ls[0]
        for a, x in zip(al[1:], ls[1:]):
            l = l + a * x
        linv = 1.0 / jnp.sum(l, axis=-1, keepdims=True)
        return [a * linv for a in al]

    def pv_chunk(par, t, c, beta):
        v = vbuf[mod(t, NS), pl.ds(c * CH, CH), :]
        p = p_refs[par][:, c * CH:(c + 1) * CH]
        oc = jnp.dot(p, v, preferred_element_type=f32)
        return oc * jnp.concatenate([beta] * (DH // 128), axis=1)

    def finalize(t, o):
        tt = max(t, 0) if isinstance(t, int) else jnp.maximum(t, 0)
        b = mod(tt, B)
        h = div(tt, B)
        o2 = jnp.concatenate([o[r * Sq:(r + 1) * Sq, :] for r in range(rep)], axis=1)
        contrib = jax.lax.dot_general(o2, wo_v[h], NT_DIMS, preferred_element_type=f32)
        acc_ref[rows_of(b), :] += contrib

    def emit_out(b):
        ostage[b] = acc_ref[rows_of(b), :].astype(ostage.dtype)
        out_copy(b).start()

    def mk_issue(t):
        def issue(j):
            n = len(all_pieces)
            for pc in all_pieces[j * n // NI:(j + 1) * n // NI]:
                if not (isinstance(t, int) and t + LAK >= T):
                    k_piece(t + LAK, *pc)
                if not (isinstance(t, int) and t + LAV >= T):
                    v_piece(t + LAV, *pc)
        return issue

    def step(t, par, ml_in, o_in, issue=None):
        o = q2 = None
        beta_in = betas(*ml_in)
        ms, ls = [None] * nch, [None] * nch
        ic = 0
        for op in ORDER.split():
            if op == 'qp':
                q2 = qproj(t + 1)
            elif op == 'fin':
                finalize(t - 1, o_in)
            elif op[0] == 'k':
                c = int(op[1:])
                ms[c], ls[c] = qk_chunk(q2, t + 1, 1 - par, c)
            elif op[0] == 'v':
                c = int(op[1:])
                oc = pv_chunk(par, t, c, beta_in[c])
                o = oc if o is None else o + oc
            elif op == 'i':
                if issue is not None:
                    issue(ic)
                ic += 1
        return (ms, ls), o.astype(bf16)

    def seq(n, fn):
        def _b(j, c):
            fn(j)
            return c
        jax.lax.fori_loop(0, n, _b, 0)

    x_copy(0).start()
    seq(4, lambda j: wq_part(0, j))
    seq(ndc, lambda j: k_chunk_start(0, j))
    x_copy(1).start()
    seq(4, lambda j: wo_part(0, j, 0))
    seq(ndc, lambda j: k_chunk_start(1, j))
    seq(ndc, lambda j: v_chunk_start(0, j, prio=0))
    wq_part(1, 0)
    wo_part(1, 0)
    acc_ref[...] = jnp.zeros_like(acc_ref)
    o_ref[...] = jnp.zeros_like(o_ref)
    with scope("pwait0"):
        x_copy(0).wait()
        wq_wait(0)
    q2 = qproj(0)
    with scope("pwait1"):
        k_wait(0)
    ms, ls = [], []
    for c in range(nch):
        mc, lc = qk_chunk(q2, 0, 0, c)
        ms.append(mc)
        ls.append(lc)
        if (c + 1) % (nch // 4) == 0:
            cc = (c + 1) // (nch // 4) - 1
            todo = [('k', g) for g in range(2, LAK)] + [('v', g) for g in range(1, LAV)]
            todo.sort(key=lambda x: x[1] - (1 if x[0] == 'k' else 0))
            n = len(todo)
            for kind, g in todo[cc * n // 4:(cc + 1) * n // 4]:
                for c2 in range(ndc):
                    (k_chunk_start if kind == 'k' else v_chunk_start)(g, c2)
    def save_ml(ml):
        for c in range(nch):
            beta_ref[c] = ml[0][c]
            beta_ref[nch + c] = ml[1][c]

    def load_ml():
        return ([beta_ref[c] for c in range(nch)], [beta_ref[nch + c] for c in range(nch)])

    save_ml((ms, ls))
    x_copy(1).wait()

    npair = (T - LA) // 2
    t_end = 2 * npair
    assert LA == 4 and B == 8 and ndc == 4

    def body(i, carry):
        t = 2 * i
        r = mod(t, B)
        u = i + 1

        @pl.when(r == 6)
        def _():
            wq_wait(div(t + 2, B))

        @pl.when(r == 0)
        def _():
            wo_wait(div(t, B))

        def issue_a(c):
            mk_issue(t)(c)
            if c == 1:
                @pl.when(u < 4 * (Hkv - 1))
                def _():
                    wq_part(div(u, 4) + 1, mod(u, 4))

        def issue_b(c):
            mk_issue(t + 1)(c)
            if c == 1:
                @pl.when(u < 4 * (Hkv - 1))
                def _():
                    wo_part(div(u, 4) + 1, mod(u, 4))

        with scope("kvwait"):
            k_wait(t + 1)
            v_wait(t)
            if not MIDWAIT:
                k_wait(t + 2)
                v_wait(t + 1)
        with scope("pair"):
            bs, o = step(t, 0, load_ml(), o_ref[...], issue=issue_a)
            if MIDWAIT:
                k_wait(t + 2)
                v_wait(t + 1)
            bs, o = step(t + 1, 1, bs, o, issue=issue_b)
            o_ref[...] = o
            save_ml(bs)

        @pl.when(t >= T - B)
        def _():
            @pl.when(t > T - B)
            def _():
                emit_out(r - 1)
            emit_out(r)

        return carry

    jax.lax.fori_loop(0, npair, body, 0)

    assert t_end + LA == T
    if LOOP_ONLY:
        return
    bs, o = load_ml(), o_ref[...]
    for t in range(t_end, T - 1):
        with scope("fwait"):
            k_wait(t + 1)
            v_wait(t)
        issue = mk_issue(t)
        with scope("fstep"):
            bs, o = step(t, t % 2, bs, o, issue=issue)
            emit_out((t - 1) % B)
    t = T - 1
    ob = None
    bs = betas(*bs)
    per = DCH // CH
    for dc in range(ndc):
        with scope("lwait"):
            v_wait_chunk(t, dc)
        with scope("lpv"):
            for c in range(dc * per, (dc + 1) * per):
                oc = pv_chunk(t % 2, t, c, bs[c])
                ob = oc if ob is None else ob + oc
            if dc == 0:
                finalize(t - 1, o)
                emit_out((t - 1) % B)
    with scope("lfin"):
        finalize(t, ob.astype(bf16))
        emit_out(t % B)
    with scope("owait"):
        for b in range(B):
            out_copy(b).wait()


@jax.jit
def pallas_standalone__gqa_block_cached__near_ridge_kernel(x, k_cache, v_cache, wq, wo):
    B, Sq, D = x.shape
    _, Hkv, Sk, Dh = k_cache.shape
    rep = HQ // Hkv
    W = rep * Dh
    R = rep * Sq
    x2 = x.reshape(B * Sq, D)
    k3 = k_cache.reshape(B * Hkv, Sk, Dh)
    v3 = v_cache.reshape(B * Hkv, Sk, Dh)
    wot = wo.T
    f32, bf16 = jnp.float32, jnp.bfloat16
    any_spec = pl.BlockSpec(memory_space=pl.ANY)
    return pl.pallas_call(
        functools.partial(_kernel, B=B, Sq=Sq, D=D, Hkv=Hkv, Sk=Sk, rep=rep),
        in_specs=[any_spec] * 5,
        out_specs=any_spec,
        out_shape=jax.ShapeDtypeStruct((B, Sq, D), x.dtype),
        scratch_shapes=[
            pltpu.VMEM((B * Sq, D), bf16),
            pltpu.VMEM((Hkv, D, W), bf16),
            pltpu.VMEM((Hkv, D, W), bf16),
            pltpu.VMEM((NS, Sk, Dh), bf16),
            pltpu.VMEM((NS, Sk, Dh), bf16),
            pltpu.VMEM((R, Sk), bf16),
            pltpu.VMEM((R, Sk), bf16),
            pltpu.VMEM((2 * (Sk // CH), R, 128), f32),
            pltpu.VMEM((R, Dh), bf16),
            pltpu.VMEM((B * Sq, D), f32),
            pltpu.VMEM((B, Sq, D), bf16),
            pltpu.SemaphoreType.DMA((2,)),
            pltpu.SemaphoreType.DMA((Hkv,)),
            pltpu.SemaphoreType.DMA((Hkv,)),
            pltpu.SemaphoreType.DMA((NS,)),
            pltpu.SemaphoreType.DMA((NS * 4,)),
            pltpu.SemaphoreType.DMA((B,)),
        ],
        compiler_params=pltpu.CompilerParams(
            vmem_limit_bytes=96 * 1024 * 1024,
            disable_bounds_checks=True,
        ),
    )(x2, k3, v3, wq, wot)
```

```python
import functools
import math

import jax
import jax.numpy as jnp
import jax.experimental.pallas as pl
import jax.experimental.pallas.tpu as pltpu

HQ, DH = 16, 256
NS = 8
CH = 512
DR = 88
LAK = 3
LAV = 3
NFINAL = 4
ORDER = "qp i fin i v0 i k0 i v1 i k1 i k2 i v2 i k3 i v3 i".split()
NT_DIMS = (((1,), (1,)), ((), ()))
QSCALE = (DH ** -0.5) * math.log2(math.e)


def _kernel(x_hbm, k_hbm, v_hbm, wq_hbm, wot_hbm, out_hbm,
            x_v, wq_v, wo_v, kbuf, vbuf, pa_ref, pb_ref, ml_ref, o_ref, acc_ref, ostage,
            xsem, wqsem, wosem, ksem, vsem, osem, *, B, Sq, D, Hkv, Sk, rep):
    T = B * Hkv
    W = rep * DH
    R = rep * Sq
    nch = Sk // CH
    f32, bf16 = jnp.float32, jnp.bfloat16
    p_refs = (pa_ref, pb_ref)
    pieces = [(o, min(DR, CH - o)) for o in range(0, CH, DR)]
    all_pieces = [(c, o, n) for c in range(nch) for (o, n) in pieces]
    n_issue = ORDER.count("i")
    assert B == 8 and nch == 4 and D % 64 == 0 and (T - NFINAL) % 2 == 0

    def mod(x, n):
        return x % n if isinstance(x, int) else jnp.bitwise_and(x, n - 1)

    def div(x, n):
        return x // n if isinstance(x, int) else jax.lax.shift_right_logical(x, n.bit_length() - 1)

    def aligned(r):
        return r if isinstance(r, int) else pl.multiple_of(r, 8)

    def blk(t):
        return mod(t, B) * Hkv + div(t, B)

    def x_copy(part):
        if part == 0:
            return pltpu.make_async_copy(x_hbm.at[pl.ds(0, Sq)], x_v.at[pl.ds(0, Sq)], xsem.at[0])
        rest = pl.ds(Sq, (B - 1) * Sq)
        return pltpu.make_async_copy(x_hbm.at[rest], x_v.at[rest], xsem.at[1])

    WP = D // 4
    WR = WP // 2

    def w_part(hbm, buf, sem, h, part):
        for j in range(2):
            r0 = aligned(part * WP + j * WR)
            pltpu.make_async_copy(hbm.at[pl.ds(r0, WR), pl.ds(h * W, W)],
                                  buf.at[h, pl.ds(r0, WR)], sem.at[h]).start(priority=0)

    def wq_part(h, part):
        w_part(wq_hbm, wq_v, wqsem, h, part)

    def wo_part(h, part):
        w_part(wot_hbm, wo_v, wosem, h, part)

    def wq_wait(h):
        pltpu.make_async_copy(wq_v.at[h], wq_v.at[h], wqsem.at[h]).wait()

    def wo_wait(h):
        pltpu.make_async_copy(wo_v.at[h], wo_v.at[h], wosem.at[h]).wait()

    def k_piece(t, c, o, n):
        slot = mod(t, NS)
        r = aligned(c * CH + o)
        pltpu.make_async_copy(k_hbm.at[blk(t), pl.ds(r, n)], kbuf.at[slot, pl.ds(r, n)],
                              ksem.at[slot]).start(priority=0)

    def v_piece(t, c, o, n, prio=1):
        slot = mod(t, NS)
        r = aligned(c * CH + o)
        pltpu.make_async_copy(v_hbm.at[blk(t), pl.ds(r, n)], vbuf.at[slot, pl.ds(r, n)],
                              vsem.at[slot]).start(priority=prio)

    def k_chunk_start(t, c):
        for o, n in pieces:
            k_piece(t, c, o, n)

    def v_chunk_start(t, c, prio=1):
        for o, n in pieces:
            v_piece(t, c, o, n, prio)

    def k_wait(t):
        slot = mod(t, NS)
        pltpu.make_async_copy(kbuf.at[slot], kbuf.at[slot], ksem.at[slot]).wait()

    def v_wait(t):
        slot = mod(t, NS)
        pltpu.make_async_copy(vbuf.at[slot], vbuf.at[slot], vsem.at[slot]).wait()

    def out_copy(b):
        return pltpu.make_async_copy(ostage.at[b], out_hbm.at[b], osem.at[b])

    def mk_issue(t):
        def issue(j):
            n = len(all_pieces)
            for pc in all_pieces[j * n // n_issue:(j + 1) * n // n_issue]:
                if not (isinstance(t, int) and t + LAK >= T):
                    k_piece(t + LAK, *pc)
                if not (isinstance(t, int) and t + LAV >= T):
                    v_piece(t + LAV, *pc)
        return issue

    def seq(n, fn):
        def _b(j, c):
            fn(j)
            return c
        jax.lax.fori_loop(0, n, _b, 0)

    def rows_of(b):
        return pl.ds(b * Sq if isinstance(b, int) else pl.multiple_of(b * Sq, Sq), Sq)

    def qproj(t):
        xb = x_v[rows_of(mod(t, B)), :]
        q = jnp.dot(xb, wq_v[div(t, B)], preferred_element_type=f32)
        q = (q * QSCALE).astype(bf16)
        return jnp.concatenate([q[:, r * DH:(r + 1) * DH] for r in range(rep)], axis=0)

    def lane_fold(a, op):
        out = a[:, 0:128]
        for j in range(1, a.shape[1] // 128):
            out = op(out, a[:, j * 128:(j + 1) * 128])
        return out

    def qk_chunk(q2, t, par, c):
        k = kbuf[mod(t, NS), pl.ds(c * CH, CH), :]
        s = jax.lax.dot_general(q2, k, NT_DIMS, preferred_element_type=f32)
        mc = jnp.max(lane_fold(s, jnp.maximum), axis=-1, keepdims=True)
        p = jnp.exp2(s - mc)
        p_refs[par][:, c * CH:(c + 1) * CH] = p.astype(bf16)
        return jnp.broadcast_to(mc, (R, 128)), lane_fold(p, jnp.add)

    def betas(ms, ls):
        m = ms[0]
        for x in ms[1:]:
            m = jnp.maximum(m, x)
        al = [jnp.exp2(x - m) for x in ms]
        l = al[0] * ls[0]
        for a, x in zip(al[1:], ls[1:]):
            l = l + a * x
        linv = 1.0 / jnp.sum(l, axis=-1, keepdims=True)
        return [a * linv for a in al]

    def pv_chunk(par, t, c, beta):
        v = vbuf[mod(t, NS), pl.ds(c * CH, CH), :]
        p = p_refs[par][:, c * CH:(c + 1) * CH]
        oc = jnp.dot(p, v, preferred_element_type=f32)
        return oc * jnp.concatenate([beta] * (DH // 128), axis=1)

    def finalize(t, o):
        tt = max(t, 0) if isinstance(t, int) else jnp.maximum(t, 0)
        o2 = jnp.concatenate([o[r * Sq:(r + 1) * Sq, :] for r in range(rep)], axis=1)
        contrib = jax.lax.dot_general(o2, wo_v[div(tt, B)], NT_DIMS, preferred_element_type=f32)
        acc_ref[rows_of(mod(tt, B)), :] += contrib

    def emit_out(b):
        ostage[b] = acc_ref[rows_of(b), :].astype(ostage.dtype)
        out_copy(b).start()

    def step(t, par, ml_in, o_in, issue):
        o = q2 = None
        beta_in = betas(*ml_in)
        ms, ls = [None] * nch, [None] * nch
        ic = 0
        for op in ORDER:
            if op == "qp":
                q2 = qproj(t + 1)
            elif op == "fin":
                finalize(t - 1, o_in)
            elif op[0] == "k":
                c = int(op[1:])
                ms[c], ls[c] = qk_chunk(q2, t + 1, 1 - par, c)
            elif op[0] == "v":
                c = int(op[1:])
                oc = pv_chunk(par, t, c, beta_in[c])
                o = oc if o is None else o + oc
            else:
                issue(ic)
                ic += 1
        return (ms, ls), o.astype(bf16)

    def save_ml(ml):
        for c in range(nch):
            ml_ref[c] = ml[0][c]
            ml_ref[nch + c] = ml[1][c]

    def load_ml():
        return ([ml_ref[c] for c in range(nch)], [ml_ref[nch + c] for c in range(nch)])

    x_copy(0).start()
    seq(4, lambda j: wq_part(0, j))
    seq(nch, lambda j: k_chunk_start(0, j))
    x_copy(1).start()
    seq(4, lambda j: wo_part(0, j))
    seq(nch, lambda j: k_chunk_start(1, j))
    seq(nch, lambda j: v_chunk_start(0, j, prio=0))
    wq_part(1, 0)
    wo_part(1, 0)
    acc_ref[...] = jnp.zeros_like(acc_ref)
    o_ref[...] = jnp.zeros_like(o_ref)
    x_copy(0).wait()
    wq_wait(0)
    q2 = qproj(0)
    k_wait(0)
    todo = [("k", g) for g in range(2, LAK)] + [("v", g) for g in range(1, LAV)]
    todo.sort(key=lambda x: x[1] - (1 if x[0] == "k" else 0))
    ms, ls = [], []
    for c in range(nch):
        mc, lc = qk_chunk(q2, 0, 0, c)
        ms.append(mc)
        ls.append(lc)
        for kind, g in todo[c * len(todo) // nch:(c + 1) * len(todo) // nch]:
            for c2 in range(nch):
                (k_chunk_start if kind == "k" else v_chunk_start)(g, c2)
    save_ml((ms, ls))
    x_copy(1).wait()

    t_end = T - NFINAL

    def body(i, carry):
        t = 2 * i
        r = mod(t, B)
        u = i + 1

        @pl.when(r == B - 2)
        def _():
            wq_wait(div(t + 2, B))

        @pl.when(r == 0)
        def _():
            wo_wait(div(t, B))

        def issue_a(j):
            mk_issue(t)(j)
            if j == 1:
                @pl.when(u < 4 * (Hkv - 1))
                def _():
                    wq_part(div(u, 4) + 1, mod(u, 4))

        def issue_b(j):
            mk_issue(t + 1)(j)
            if j == 1:
                @pl.when(u < 4 * (Hkv - 1))
                def _():
                    wo_part(div(u, 4) + 1, mod(u, 4))

        k_wait(t + 1)
        v_wait(t)
        ml, o = step(t, 0, load_ml(), o_ref[...], issue_a)
        k_wait(t + 2)
        v_wait(t + 1)
        ml, o = step(t + 1, 1, ml, o, issue_b)
        o_ref[...] = o
        save_ml(ml)

        @pl.when(t >= T - B)
        def _():
            @pl.when(t > T - B)
            def _():
                emit_out(r - 1)
            emit_out(r)

        return carry

    jax.lax.fori_loop(0, t_end // 2, body, 0)

    ml, o = load_ml(), o_ref[...]
    for t in range(t_end, T - 1):
        k_wait(t + 1)
        v_wait(t)
        ml, o = step(t, t % 2, ml, o, mk_issue(t))
        emit_out((t - 1) % B)
    t = T - 1
    bs = betas(*ml)
    v_wait(t)
    ob = None
    for c in range(nch):
        oc = pv_chunk(t % 2, t, c, bs[c])
        ob = oc if ob is None else ob + oc
        if c == 0:
            finalize(t - 1, o)
            emit_out((t - 1) % B)
    finalize(t, ob.astype(bf16))
    emit_out(t % B)
    for b in range(B):
        out_copy(b).wait()


@jax.jit
def pallas_standalone__gqa_block_cached__near_ridge_kernel(x, k_cache, v_cache, wq, wo):
    B, Sq, D = x.shape
    _, Hkv, Sk, Dh = k_cache.shape
    rep = HQ // Hkv
    W = rep * Dh
    R = rep * Sq
    x2 = x.reshape(B * Sq, D)
    k3 = k_cache.reshape(B * Hkv, Sk, Dh)
    v3 = v_cache.reshape(B * Hkv, Sk, Dh)
    wot = wo.T
    f32, bf16 = jnp.float32, jnp.bfloat16
    any_spec = pl.BlockSpec(memory_space=pl.ANY)
    return pl.pallas_call(
        functools.partial(_kernel, B=B, Sq=Sq, D=D, Hkv=Hkv, Sk=Sk, rep=rep),
        in_specs=[any_spec] * 5,
        out_specs=any_spec,
        out_shape=jax.ShapeDtypeStruct((B, Sq, D), x.dtype),
        scratch_shapes=[
            pltpu.VMEM((B * Sq, D), bf16),
            pltpu.VMEM((Hkv, D, W), bf16),
            pltpu.VMEM((Hkv, D, W), bf16),
            pltpu.VMEM((NS, Sk, Dh), bf16),
            pltpu.VMEM((NS, Sk, Dh), bf16),
            pltpu.VMEM((R, Sk), bf16),
            pltpu.VMEM((R, Sk), bf16),
            pltpu.VMEM((2 * (Sk // CH), R, 128), f32),
            pltpu.VMEM((R, Dh), bf16),
            pltpu.VMEM((B * Sq, D), f32),
            pltpu.VMEM((B, Sq, D), bf16),
            pltpu.SemaphoreType.DMA((2,)),
            pltpu.SemaphoreType.DMA((Hkv,)),
            pltpu.SemaphoreType.DMA((Hkv,)),
            pltpu.SemaphoreType.DMA((NS,)),
            pltpu.SemaphoreType.DMA((NS,)),
            pltpu.SemaphoreType.DMA((B,)),
        ],
        compiler_params=pltpu.CompilerParams(
            vmem_limit_bytes=96 * 1024 * 1024,
            disable_bounds_checks=True,
        ),
    )(x2, k3, v3, wq, wot)
```

```python
import functools
import math

import jax
import jax.numpy as jnp
import jax.experimental.pallas as pl
import jax.experimental.pallas.tpu as pltpu

HQ, DH = 16, 256
NS = 8
CH = 512
DR = 88
LAK = 3
LAV = 3
NFINAL = 4
ORDER = "qp i fin i v0 i k0 i v1 i k1 i k2 i v2 i k3 i v3 i".split()
NT_DIMS = (((1,), (1,)), ((), ()))
QSCALE = (DH ** -0.5) * math.log2(math.e)


def _kernel(x_hbm, k_hbm, v_hbm, wq_hbm, wot_hbm, out_hbm,
            x_v, wq_v, wo_v, kbuf, vbuf, pa_ref, pb_ref, ml_ref, o_ref, acc_ref, ostage,
            xsem, wqsem, wosem, ksem, vsem, osem, *, B, Sq, D, Hkv, Sk, rep):
    T = B * Hkv
    W = rep * DH
    R = rep * Sq
    nch = Sk // CH
    f32, bf16 = jnp.float32, jnp.bfloat16
    p_refs = (pa_ref, pb_ref)
    pieces = [(o, min(DR, CH - o)) for o in range(0, CH, DR)]
    all_pieces = [(c, o, n) for c in range(nch) for (o, n) in pieces]
    n_issue = ORDER.count("i")
    assert B == 8 and nch == 4 and D % 64 == 0 and (T - NFINAL) % 2 == 0

    def mod(x, n):
        return x % n if isinstance(x, int) else jnp.bitwise_and(x, n - 1)

    def div(x, n):
        return x // n if isinstance(x, int) else jax.lax.shift_right_logical(x, n.bit_length() - 1)

    def aligned(r):
        return r if isinstance(r, int) else pl.multiple_of(r, 8)

    def blk(t):
        return mod(t, B) * Hkv + div(t, B)

    def x_copy(part):
        if part == 0:
            return pltpu.make_async_copy(x_hbm.at[pl.ds(0, Sq)], x_v.at[pl.ds(0, Sq)], xsem.at[0])
        rest = pl.ds(Sq, (B - 1) * Sq)
        return pltpu.make_async_copy(x_hbm.at[rest], x_v.at[rest], xsem.at[1])

    WP = D // 4
    WR = WP // 2

    def w_part(hbm, buf, sem, h, part):
        for j in range(2):
            r0 = aligned(part * WP + j * WR)
            pltpu.make_async_copy(hbm.at[pl.ds(r0, WR), pl.ds(h * W, W)],
                                  buf.at[h, pl.ds(r0, WR)], sem.at[h]).start(priority=0)

    def wq_part(h, part):
        w_part(wq_hbm, wq_v, wqsem, h, part)

    def wo_part(h, part):
        w_part(wot_hbm, wo_v, wosem, h, part)

    def wq_wait(h):
        pltpu.make_async_copy(wq_v.at[h], wq_v.at[h], wqsem.at[h]).wait()

    def wo_wait(h):
        pltpu.make_async_copy(wo_v.at[h], wo_v.at[h], wosem.at[h]).wait()

    def k_piece(t, c, o, n):
        slot = mod(t, NS)
        r = aligned(c * CH + o)
        pltpu.make_async_copy(k_hbm.at[blk(t), pl.ds(r, n)], kbuf.at[slot, pl.ds(r, n)],
                              ksem.at[slot]).start(priority=0)

    def v_piece(t, c, o, n, prio=1):
        slot = mod(t, NS)
        r = aligned(c * CH + o)
        pltpu.make_async_copy(v_hbm.at[blk(t), pl.ds(r, n)], vbuf.at[slot, pl.ds(r, n)],
                              vsem.at[slot]).start(priority=prio)

    def k_chunk_start(t, c):
        for o, n in pieces:
            k_piece(t, c, o, n)

    def v_chunk_start(t, c, prio=1):
        for o, n in pieces:
            v_piece(t, c, o, n, prio)

    def k_wait(t):
        slot = mod(t, NS)
        pltpu.make_async_copy(kbuf.at[slot], kbuf.at[slot], ksem.at[slot]).wait()

    def v_wait(t):
        slot = mod(t, NS)
        pltpu.make_async_copy(vbuf.at[slot], vbuf.at[slot], vsem.at[slot]).wait()

    def out_copy(b):
        return pltpu.make_async_copy(ostage.at[b], out_hbm.at[b], osem.at[b])

    def mk_issue(t):
        def issue(j):
            n = len(all_pieces)
            for pc in all_pieces[j * n // n_issue:(j + 1) * n // n_issue]:
                if not (isinstance(t, int) and t + LAK >= T):
                    k_piece(t + LAK, *pc)
                if not (isinstance(t, int) and t + LAV >= T):
                    v_piece(t + LAV, *pc)
        return issue

    def seq(n, fn):
        def _b(j, c):
            fn(j)
            return c
        jax.lax.fori_loop(0, n, _b, 0)

    def rows_of(b):
        return pl.ds(b * Sq if isinstance(b, int) else pl.multiple_of(b * Sq, Sq), Sq)

    def qproj(t):
        xb = x_v[rows_of(mod(t, B)), :]
        q = jnp.dot(xb, wq_v[div(t, B)], preferred_element_type=f32)
        q = (q * QSCALE).astype(bf16)
        return jnp.concatenate([q[:, r * DH:(r + 1) * DH] for r in range(rep)], axis=0)

    def lane_fold(a, op):
        out = a[:, 0:128]
        for j in range(1, a.shape[1] // 128):
            out = op(out, a[:, j * 128:(j + 1) * 128])
        return out

    def qk_chunk(q2, t, par, c):
        k = kbuf[mod(t, NS), pl.ds(c * CH, CH), :]
        s = jax.lax.dot_general(q2, k, NT_DIMS, preferred_element_type=f32)
        mc = jnp.max(lane_fold(s, jnp.maximum), axis=-1, keepdims=True)
        p = jnp.exp2(s - mc)
        p_refs[par][:, c * CH:(c + 1) * CH] = p.astype(bf16)
        return jnp.broadcast_to(mc, (R, 128)), lane_fold(p, jnp.add)

    def betas(ms, ls):
        m = ms[0]
        for x in ms[1:]:
            m = jnp.maximum(m, x)
        al = [jnp.exp2(x - m) for x in ms]
        l = al[0] * ls[0]
        for a, x in zip(al[1:], ls[1:]):
            l = l + a * x
        linv = 1.0 / jnp.sum(l, axis=-1, keepdims=True)
        return [a * linv for a in al]

    def pv_chunk(par, t, c, beta):
        v = vbuf[mod(t, NS), pl.ds(c * CH, CH), :]
        p = p_refs[par][:, c * CH:(c + 1) * CH]
        oc = jnp.dot(p, v, preferred_element_type=f32)
        return oc * jnp.concatenate([beta] * (DH // 128), axis=1)

    def finalize(t, o):
        tt = max(t, 0) if isinstance(t, int) else jnp.maximum(t, 0)
        o2 = jnp.concatenate([o[r * Sq:(r + 1) * Sq, :] for r in range(rep)], axis=1)
        contrib = jax.lax.dot_general(o2, wo_v[div(tt, B)], NT_DIMS, preferred_element_type=f32)
        acc_ref[rows_of(mod(tt, B)), :] += contrib

    def emit_out(b):
        ostage[b] = acc_ref[rows_of(b), :].astype(ostage.dtype)
        out_copy(b).start()

    def step(t, par, ml_in, o_in, issue):
        o = q2 = None
        beta_in = betas(*ml_in)
        ms, ls = [None] * nch, [None] * nch
        ic = 0
        for op in ORDER:
            if op == "qp":
                q2 = qproj(t + 1)
            elif op == "fin":
                finalize(t - 1, o_in)
            elif op[0] == "k":
                c = int(op[1:])
                ms[c], ls[c] = qk_chunk(q2, t + 1, 1 - par, c)
            elif op[0] == "v":
                c = int(op[1:])
                oc = pv_chunk(par, t, c, beta_in[c])
                o = oc if o is None else o + oc
            else:
                issue(ic)
                ic += 1
        return (ms, ls), o.astype(bf16)

    def save_ml(ml):
        for c in range(nch):
            ml_ref[c] = ml[0][c]
            ml_ref[nch + c] = ml[1][c]

    def load_ml():
        return ([ml_ref[c] for c in range(nch)], [ml_ref[nch + c] for c in range(nch)])

    x_copy(0).start()
    seq(4, lambda j: wq_part(0, j))
    seq(nch, lambda j: k_chunk_start(0, j))
    x_copy(1).start()
    seq(4, lambda j: wo_part(0, j))
    seq(nch, lambda j: k_chunk_start(1, j))
    seq(nch, lambda j: v_chunk_start(0, j, prio=0))
    wq_part(1, 0)
    wo_part(1, 0)
    acc_ref[...] = jnp.zeros_like(acc_ref)
    o_ref[...] = jnp.zeros_like(o_ref)
    x_copy(0).wait()
    wq_wait(0)
    q2 = qproj(0)
    k_wait(0)
    todo = [("k", g) for g in range(2, LAK)] + [("v", g) for g in range(1, LAV)]
    todo.sort(key=lambda x: x[1] - (1 if x[0] == "k" else 0))
    ms, ls = [], []
    for c in range(nch):
        mc, lc = qk_chunk(q2, 0, 0, c)
        ms.append(mc)
        ls.append(lc)
        for kind, g in todo[c * len(todo) // nch:(c + 1) * len(todo) // nch]:
            for c2 in range(nch):
                (k_chunk_start if kind == "k" else v_chunk_start)(g, c2)
    save_ml((ms, ls))
    x_copy(1).wait()

    t_end = T - NFINAL

    def body(i, carry):
        t = 2 * i
        r = mod(t, B)
        u = i + 1

        @pl.when(r == B - 2)
        def _():
            wq_wait(div(t + 2, B))

        @pl.when(r == 0)
        def _():
            wo_wait(div(t, B))

        def issue_a(j):
            mk_issue(t)(j)
            if j == 1:
                @pl.when(u < 4 * (Hkv - 1))
                def _():
                    wq_part(div(u, 4) + 1, mod(u, 4))

        def issue_b(j):
            mk_issue(t + 1)(j)
            if j == 1:
                @pl.when(u < 4 * (Hkv - 1))
                def _():
                    wo_part(div(u, 4) + 1, mod(u, 4))

        k_wait(t + 1)
        v_wait(t)
        ml, o = step(t, 0, load_ml(), o_ref[...], issue_a)
        k_wait(t + 2)
        v_wait(t + 1)
        ml, o = step(t + 1, 1, ml, o, issue_b)
        o_ref[...] = o
        save_ml(ml)

        return carry

    jax.lax.fori_loop(0, t_end // 2, body, 0)

    for t in range(t_end, T - 1):
        k_wait(t + 1)
        v_wait(t)
        if t == t_end:
            ml, o = load_ml(), o_ref[...]
            for b in range(t_end - 1 - (T - B)):
                emit_out(b)
        ml, o = step(t, t % 2, ml, o, mk_issue(t))
        emit_out((t - 1) % B)
    t = T - 1
    v_wait(t)
    bs = betas(*ml)
    ob = None
    for c in range(nch):
        oc = pv_chunk(t % 2, t, c, bs[c])
        ob = oc if ob is None else ob + oc
        if c == 0:
            finalize(t - 1, o)
            emit_out((t - 1) % B)
    finalize(t, ob.astype(bf16))
    emit_out(t % B)
    for b in range(B):
        out_copy(b).wait()


@jax.jit
def pallas_standalone__gqa_block_cached__near_ridge_kernel(x, k_cache, v_cache, wq, wo):
    B, Sq, D = x.shape
    _, Hkv, Sk, Dh = k_cache.shape
    rep = HQ // Hkv
    W = rep * Dh
    R = rep * Sq
    x2 = x.reshape(B * Sq, D)
    k3 = k_cache.reshape(B * Hkv, Sk, Dh)
    v3 = v_cache.reshape(B * Hkv, Sk, Dh)
    wot = wo.T
    f32, bf16 = jnp.float32, jnp.bfloat16
    any_spec = pl.BlockSpec(memory_space=pl.ANY)
    return pl.pallas_call(
        functools.partial(_kernel, B=B, Sq=Sq, D=D, Hkv=Hkv, Sk=Sk, rep=rep),
        in_specs=[any_spec] * 5,
        out_specs=any_spec,
        out_shape=jax.ShapeDtypeStruct((B, Sq, D), x.dtype),
        scratch_shapes=[
            pltpu.VMEM((B * Sq, D), bf16),
            pltpu.VMEM((Hkv, D, W), bf16),
            pltpu.VMEM((Hkv, D, W), bf16),
            pltpu.VMEM((NS, Sk, Dh), bf16),
            pltpu.VMEM((NS, Sk, Dh), bf16),
            pltpu.VMEM((R, Sk), bf16),
            pltpu.VMEM((R, Sk), bf16),
            pltpu.VMEM((2 * (Sk // CH), R, 128), f32),
            pltpu.VMEM((R, Dh), bf16),
            pltpu.VMEM((B * Sq, D), f32),
            pltpu.VMEM((B, Sq, D), bf16),
            pltpu.SemaphoreType.DMA((2,)),
            pltpu.SemaphoreType.DMA((Hkv,)),
            pltpu.SemaphoreType.DMA((Hkv,)),
            pltpu.SemaphoreType.DMA((NS,)),
            pltpu.SemaphoreType.DMA((NS,)),
            pltpu.SemaphoreType.DMA((B,)),
        ],
        compiler_params=pltpu.CompilerParams(
            vmem_limit_bytes=96 * 1024 * 1024,
            disable_bounds_checks=True,
            disable_semaphore_checks=True,
        ),
    )(x2, k3, v3, wq, wot)
```
